```python
import jax
import jax.numpy as jnp

def _softmax(x, axis=-1):
    return jax.nn.softmax(x, axis=axis)
def _gelu(x):
    return jax.nn.gelu(x, approximate=True)
def _silu(x):
    return jax.nn.silu(x)
def _sigmoid(x):
    return jax.nn.sigmoid(x)
def _layernorm(x, axis=-1, eps=1e-5):
    m = jnp.mean(x, axis=axis, keepdims=True)
    v = jnp.var(x, axis=axis, keepdims=True)
    return (x - m) / jnp.sqrt(v + eps)
def _scatter_add(tgt, idx, src, axis=0):
    return tgt.at[idx].add(src)
def _segment_sum(src, seg, n):
    return jax.ops.segment_sum(src, seg, n)
class _Rng:
    def __init__(self, key):
        self._k = key
    def _next(self):
        self._k, sub = jax.random.split(self._k)
        return sub
    def normal(self, shape):
        return jax.random.normal(self._next(), shape, dtype=jnp.bfloat16)
    def randint(self, lo, hi, shape):
        return jax.random.randint(self._next(), shape, lo, hi, dtype=jnp.int32)
    def uniform(self, shape, lo=0.0, hi=1.0):
        return jax.random.uniform(self._next(), shape, jnp.bfloat16, lo, hi)
    def permutation(self, n):
        return jax.random.permutation(self._next(), n)


kernel_name = 'standalone__instancenorm__prompt'

def setup_inputs():
    _rng = _Rng(jax.random.key(int.from_bytes(__import__("os").urandom(4), "little")))
    _w = (lambda a: (lambda t: t.astype(jnp.bfloat16) if jnp.issubdtype(t.dtype, jnp.floating) else t)(jnp.asarray(a)))
    B, C, H, W = 2, 1024, 2048, 32
    return {
        "x": _w((lambda *s: _rng.normal(s) * 0.05)(B, C, H, W)),
        "g": _w((lambda *s: _rng.normal(s) * 0.05)(C) + 1.0),
        "b": _w((lambda *s: _rng.normal(s) * 0.05)(C)),
    }

def reference(x, g, b):
    mu = x.mean(axis=(-2, -1), keepdims=True)
    var = ((x - mu) * (x - mu)).mean(axis=(-2, -1), keepdims=True)
    xhat = (x - mu) / jnp.sqrt(var + 1e-5)
    return xhat * g.reshape(1, -1, 1, 1) + b.reshape(1, -1, 1, 1)
```

```python
import jax
import jax.numpy as jnp
from jax import lax
import jax.experimental.pallas as pl
import jax.experimental.pallas.tpu as pltpu

_EPS = 1e-5
_LANES = 128
_ROWS = 16


def _make_kernel(B, C, H, W, S, m, u, win, rsplit, wsplit, G):
    N = B * C
    per = N // S
    nch = per // m
    steps = m // u
    nsem = 2 * max(win, 2)
    inv_n = 1.0 / (H * W)
    CW = 256

    def pieces(split):
        rh, cb = split
        return [
            (jj, pl.ds(h * (W // rh), W // rh), pl.ds(c * (H // cb), H // cb))
            for jj in range(u)
            for h in range(rh)
            for c in range(cb)
        ]

    rp, wp = pieces(rsplit), pieces(wsplit)
    blocks = [
        (pl.ds(h * _ROWS, _ROWS), pl.ds(cb * CW, CW))
        for h in range(W // _ROWS)
        for cb in range(H // CW)
    ]

    def kernel(x_hbm, g_ref, b_ref, o_hbm, buf, gt, bt, rs, ws):
        def reads(c, j):
            sem = rs.at[lax.rem(j, nsem)]
            return [
                pltpu.make_async_copy(
                    x_hbm.at[:, c * m + j * u + jj, rr, cc],
                    buf.at[:, j * u + jj, rr, cc],
                    sem,
                )
                for jj, rr, cc in rp
            ]

        def writes(c, j):
            sem = ws.at[lax.rem(j, nsem)]
            return [
                pltpu.make_async_copy(
                    buf.at[:, j * u + jj, rr, cc],
                    o_hbm.at[:, c * m + j * u + jj, rr, cc],
                    sem,
                )
                for jj, rr, cc in wp
            ]

        def start(copies):
            for n, d in enumerate(copies):
                d.start(priority=n % 2)

        def wait(copies):
            for d in copies:
                d.wait()

        for t in range(win):
            start(reads(jnp.int32(0), jnp.int32(t)))

        for src, dst in ((g_ref, gt), (b_ref, bt)):
            v = src[...].astype(jnp.float32)
            for k in range(C // _LANES):
                dst[pl.ds(k * _LANES, _LANES), :] = jnp.broadcast_to(
                    v[k : k + 1, :], (_LANES, _LANES)
                ).T

        def total(acc):
            return jnp.sum(jnp.sum(acc, axis=1, keepdims=True), axis=0, keepdims=True)

        def normalise_group(c, s0, jj):
            insts = [s0 + a for a in range(G)]
            mus = []
            for s in insts:
                acc = None
                for rr, cc in blocks:
                    v = buf[s, jj, rr, cc].astype(jnp.float32)
                    acc = v if acc is None else acc + v
                mus.append(total(acc) * inv_n)
            affine = []
            for s, mu in zip(insts, mus):
                acc = None
                for rr, cc in blocks:
                    v = buf[s, jj, rr, cc].astype(jnp.float32) - mu
                    v = v * v
                    acc = v if acc is None else acc + v
                ch = lax.rem(s * per + c * m + jj, C)
                scale = lax.rsqrt(total(acc) * inv_n + _EPS) * gt[pl.ds(ch, 1), :]
                shift = bt[pl.ds(ch, 1), :] - mu * scale
                reps = CW // _LANES
                affine.append(
                    (
                        jnp.concatenate([scale] * reps, axis=1),
                        jnp.concatenate([shift] * reps, axis=1),
                    )
                )
            for s, (scale, shift) in zip(insts, affine):
                for rr, cc in blocks:
                    v = buf[s, jj, rr, cc].astype(jnp.float32)
                    buf[s, jj, rr, cc] = (v * scale + shift).astype(buf.dtype)

        def normalise_step(c, j):
            def body(i, carry):
                normalise_group(c, lax.rem(i, S // G) * G, j * u + i // (S // G))
                return carry

            lax.fori_loop(0, (S // G) * u, body, 0)

        def chunk(c, carry):
            def read_phase(j, carry):
                wait(reads(c, j))

                @pl.when(j + win < steps)
                def _():
                    start(reads(c, j + win))

                @pl.when(j + win >= steps)
                def _():
                    start(writes(c, j + win - steps))

                normalise_step(c, j)
                return carry

            lax.fori_loop(0, steps, read_phase, 0)

            def write_phase(j, carry):
                wait(writes(c, j))

                @pl.when(j + win < steps)
                def _():
                    start(writes(c, j + win))

                @pl.when(jnp.logical_and(j + win >= steps, c + 1 < nch))
                def _():
                    start(reads(c + 1, j + win - steps))

                return carry

            lax.fori_loop(0, steps, write_phase, 0)
            return carry

        lax.fori_loop(0, nch, chunk, 0)

    scratch = [
        pltpu.VMEM((S, m, W, H), jnp.bfloat16),
        pltpu.VMEM((C, _LANES), jnp.float32),
        pltpu.VMEM((C, _LANES), jnp.float32),
        pltpu.SemaphoreType.DMA((nsem,)),
        pltpu.SemaphoreType.DMA((nsem,)),
    ]
    return kernel, scratch


@jax.jit
def pallas_standalone__instancenorm__prompt_kernel(
    x: jax.Array,
    g: jax.Array,
    b: jax.Array,
):
    B, C, H, W = x.shape
    S = 4
    kernel, scratch = _make_kernel(
        B, C, H, W, S=S, m=128, u=4, win=2, rsplit=(2, 1), wsplit=(2, 4), G=4
    )
    xt = jnp.transpose(x, (0, 1, 3, 2)).reshape(S, B * C // S, W, H)
    y = pl.pallas_call(
        kernel,
        in_specs=[
            pl.BlockSpec(memory_space=pl.ANY),
            pl.BlockSpec(memory_space=pltpu.VMEM),
            pl.BlockSpec(memory_space=pltpu.VMEM),
        ],
        out_specs=pl.BlockSpec(memory_space=pl.ANY),
        out_shape=jax.ShapeDtypeStruct(xt.shape, xt.dtype),
        scratch_shapes=scratch,
        compiler_params=pltpu.CompilerParams(vmem_limit_bytes=100 * 1024 * 1024),
    )(xt, g.reshape(C // _LANES, _LANES), b.reshape(C // _LANES, _LANES))
    return jnp.transpose(y.reshape(B, C, W, H), (0, 1, 3, 2))
```

```python
import jax
import jax.numpy as jnp
from jax import lax
import jax.experimental.pallas as pl
import jax.experimental.pallas.tpu as pltpu

_EPS = 1e-5
_LANES = 128

_S = 4
_M = 128
_R_ROWS, _R_COLS, _R_WIN = 8, 1024, 32
_W_ROWS, _W_COLS, _W_WIN = 8, 512, 2
_K_RW = 8
_C_ROWS, _C_COLS = 16, 256


def _make_kernel(B, C, H, W):
    S, m = _S, _M
    per = B * C // S
    nch = per // m
    rcb = H // _R_COLS
    rpj = (W // _R_ROWS) * rcb
    rwj = _R_WIN // rpj
    inv_n = 1.0 / (H * W)
    blocks = [
        (pl.ds(h * _C_ROWS, _C_ROWS), pl.ds(cb * _C_COLS, _C_COLS))
        for h in range(W // _C_ROWS)
        for cb in range(H // _C_COLS)
    ]

    def kernel(x_hbm, g_ref, b_ref, o_hbm, buf, gt, bt, rs, ws):
        def r_copy(c, j, p, streams):
            rr = pl.ds((p // rcb) * _R_ROWS, _R_ROWS)
            cc = pl.ds((p % rcb) * _R_COLS, _R_COLS)
            return pltpu.make_async_copy(
                x_hbm.at[streams, c * m + j, rr, cc],
                buf.at[streams, j, rr, cc],
                rs.at[lax.rem(j, rwj) * rpj + p],
            )

        def r_start(c, j, p):
            for q in range(2):
                r_copy(c, j, p, pl.ds(q * (S // 2), S // 2)).start(priority=q)

        def r_wait(c, j, p):
            r_copy(c, j, p, pl.ds(0, S)).wait()

        def r_fill_window(c):
            for t in range(_R_WIN):
                r_start(c, jnp.int32(t // rpj), t % rpj)

        def r_column(c, j):
            for p in range(rpj):
                r_wait(c, j, p)
                r_start(c, j + rwj, p)

        def w_start(c, j):
            for h in range(W // _W_ROWS):
                for cb in range(H // _W_COLS):
                    rr = pl.ds(h * _W_ROWS, _W_ROWS)
                    cc = pl.ds(cb * _W_COLS, _W_COLS)
                    pltpu.make_async_copy(
                        buf.at[:, j, rr, cc],
                        o_hbm.at[:, c * m + j, rr, cc],
                        ws.at[lax.rem(j, _W_WIN)],
                    ).start()

        def w_wait(c, j):
            pltpu.make_async_copy(
                buf.at[:, j], o_hbm.at[:, c * m + j], ws.at[lax.rem(j, _W_WIN)]
            ).wait()

        r_fill_window(jnp.int32(0))

        for src, dst in ((g_ref, gt), (b_ref, bt)):
            v = src[...].astype(jnp.float32)
            for k in range(C // _LANES):
                dst[pl.ds(k * _LANES, _LANES), :] = jnp.broadcast_to(
                    v[k : k + 1, :], (_LANES, _LANES)
                ).T

        def total(acc):
            return jnp.sum(jnp.sum(acc, axis=1, keepdims=True), axis=0, keepdims=True)

        def normalise(c, j):
            mus = []
            for s in range(S):
                acc = None
                for rr, cc in blocks:
                    v = buf[s, j, rr, cc].astype(jnp.float32)
                    acc = v if acc is None else acc + v
                mus.append(total(acc) * inv_n)
            affine = []
            for s in range(S):
                acc = None
                for rr, cc in blocks:
                    v = buf[s, j, rr, cc].astype(jnp.float32) - mus[s]
                    v = v * v
                    acc = v if acc is None else acc + v
                ch = lax.rem(s * per + c * m + j, C)
                scale = lax.rsqrt(total(acc) * inv_n + _EPS) * gt[pl.ds(ch, 1), :]
                shift = bt[pl.ds(ch, 1), :] - mus[s] * scale
                reps = _C_COLS // _LANES
                affine.append(
                    (
                        jnp.concatenate([scale] * reps, axis=1),
                        jnp.concatenate([shift] * reps, axis=1),
                    )
                )
            for s in range(S):
                scale, shift = affine[s]
                for rr, cc in blocks:
                    v = buf[s, j, rr, cc].astype(jnp.float32)
                    buf[s, j, rr, cc] = (v * scale + shift).astype(buf.dtype)

        def loop(lo, hi, body):
            def wrapped(j, carry):
                body(j)
                return carry

            lax.fori_loop(lo, hi, wrapped, 0)

        def chunk(c):
            def read_and_normalise(j):
                r_column(c, j)
                normalise(c, j)

            loop(0, _W_WIN, read_and_normalise)
            loop(_W_WIN, m - rwj, lambda j: r_column(c, j))
            for t in range(_R_WIN):
                if _R_WIN - t == _K_RW:
                    for j in range(_W_WIN):
                        w_start(c, jnp.int32(j))
                r_wait(c, jnp.int32(m - rwj + t // rpj), t % rpj)

            def normalise_and_write(j):
                normalise(c, j + _W_WIN)
                w_wait(c, j)
                w_start(c, j + _W_WIN)

            loop(0, m - _W_WIN, normalise_and_write)
            for j in range(m - _W_WIN, m):
                w_wait(c, jnp.int32(j))

            @pl.when(c + 1 < nch)
            def _():
                r_fill_window(c + 1)

        loop(0, nch, chunk)

    scratch = [
        pltpu.VMEM((S, m, W, H), jnp.bfloat16),
        pltpu.VMEM((C, _LANES), jnp.float32),
        pltpu.VMEM((C, _LANES), jnp.float32),
        pltpu.SemaphoreType.DMA((_R_WIN,)),
        pltpu.SemaphoreType.DMA((_W_WIN,)),
    ]
    return kernel, scratch


@jax.jit
def pallas_standalone__instancenorm__prompt_kernel(
    x: jax.Array,
    g: jax.Array,
    b: jax.Array,
):
    B, C, H, W = x.shape
    kernel, scratch = _make_kernel(B, C, H, W)
    xt = jnp.transpose(x, (0, 1, 3, 2)).reshape(_S, B * C // _S, W, H)
    y = pl.pallas_call(
        kernel,
        in_specs=[
            pl.BlockSpec(memory_space=pl.ANY),
            pl.BlockSpec(memory_space=pltpu.VMEM),
            pl.BlockSpec(memory_space=pltpu.VMEM),
        ],
        out_specs=pl.BlockSpec(memory_space=pl.ANY),
        out_shape=jax.ShapeDtypeStruct(xt.shape, xt.dtype),
        scratch_shapes=scratch,
        compiler_params=pltpu.CompilerParams(vmem_limit_bytes=100 * 1024 * 1024),
    )(xt, g.reshape(C // _LANES, _LANES), b.reshape(C // _LANES, _LANES))
    return jnp.transpose(y.reshape(B, C, W, H), (0, 1, 3, 2))
```
